```python
import os as _os
_os.environ.setdefault('JAX_PLATFORMS', 'cpu')
import jax
import jax.numpy as jnp

def _softmax(x, axis=-1):
    return jax.nn.softmax(x, axis=axis)

def _gelu(x):
    return jax.nn.gelu(x, approximate=True)

def _silu(x):
    return jax.nn.silu(x)

def _sigmoid(x):
    return jax.nn.sigmoid(x)

def _layernorm(x, axis=-1, eps=1e-05):
    m = jnp.mean(x, axis=axis, keepdims=True)
    v = jnp.var(x, axis=axis, keepdims=True)
    return (x - m) / jnp.sqrt(v + eps)

def _scatter_add(tgt, idx, src, axis=0):
    return tgt.at[idx].add(src)

def _segment_sum(src, seg, n):
    return jax.ops.segment_sum(src, seg, n)

class _Rng:

    def __init__(self, key):
        self._k = key

    def _next(self):
        self._k, sub = jax.random.split(self._k)
        return sub

    def normal(self, shape):
        return jax.random.normal(self._next(), shape, dtype=jnp.bfloat16)

    def randint(self, lo, hi, shape):
        return jax.random.randint(self._next(), shape, lo, hi, dtype=jnp.int32)

    def uniform(self, shape, lo=0.0, hi=1.0):
        return jax.random.uniform(self._next(), shape, jnp.bfloat16, lo, hi)

    def permutation(self, n):
        return jax.random.permutation(self._next(), n)
kernel_name = 'sequential_preLN__memory_aug_recurrent_mem_tr__swiglu_ffn__prompt'

def setup_inputs():
    _rng = _Rng(jax.random.key(int.from_bytes(__import__("os").urandom(4), "little")))
    _w = lambda a: (lambda t: t.astype(jnp.bfloat16) if jnp.issubdtype(t.dtype, jnp.floating) else t)(jnp.asarray(a))

    def _A_setup():
        B, S, Dm = (1, 2048, 640)
        H, Dh = (32, 192)
        M, seg = (8, 32)
        seg = min(seg, S)
        S = S // seg * seg
        return {'x': _w((lambda *s: _rng.normal(s) * 0.05)(B, S, Dm)), 'mem0': _w((lambda *s: _rng.normal(s) * 0.1)(B, M, Dm)), 'Wq': _w((lambda *s: _rng.normal(s) * 1.6)(Dm, H, Dh) * Dm ** (-0.5)), 'Wk': _w((lambda *s: _rng.normal(s) * 1.6)(Dm, H, Dh) * Dm ** (-0.5)), 'Wv': _w((lambda *s: _rng.normal(s) * 0.1)(Dm, H, Dh) * Dm ** (-0.5)), 'Wo': _w((lambda *s: _rng.normal(s) * 0.1)(H, Dh, Dm) * (H * Dh) ** (-0.5)), 'seg_len': seg}
    _A_in = _A_setup()

    def _B_setup():
        B, S, D, F = (1, 2048, 640, 1536)
        return {'x': _w((lambda *s: _rng.normal(s) * 0.05)(B, S, D)), 'w_gate': _w((lambda *s: _rng.normal(s) * 0.05)(D, F)), 'w_up': _w((lambda *s: _rng.normal(s) * 0.05)(D, F)), 'w_down': _w((lambda *s: _rng.normal(s) * 0.05)(F, D))}
    _B_in = _B_setup()
    return {'A_x': _A_in['x'], 'A_mem0': _A_in['mem0'], 'A_Wq': _A_in['Wq'], 'A_Wk': _A_in['Wk'], 'A_Wv': _A_in['Wv'], 'A_Wo': _A_in['Wo'], 'A_seg_len': _A_in['seg_len'], 'B_x': _B_in['x'], 'B_w_gate': _B_in['w_gate'], 'B_w_up': _B_in['w_up'], 'B_w_down': _B_in['w_down']}

def reference(A_x, A_mem0, A_Wq, A_Wk, A_Wv, A_Wo, A_seg_len, B_x, B_w_gate, B_w_up, B_w_down):

    def _A_ref(x, mem0, Wq, Wk, Wv, Wo, seg_len):
        B, S, Dm = x.shape
        H, Dh = (Wq.shape[1], Wq.shape[2])
        M = mem0.shape[1]
        scale = Dh ** (-0.5)
        n_seg = S // seg_len
        L = M + seg_len
        idx = jnp.arange(L)
        mask = (idx[:, None] < M) | (idx[:, None] >= idx[None, :])
        mem = mem0
        outs = []
        for s in range(n_seg):
            xs = x[:, s * seg_len:(s + 1) * seg_len, :].copy()
            h = jnp.concatenate([mem, xs], axis=1)
            q = jnp.einsum('btd,dhe->bhte', h, Wq)
            k = jnp.einsum('btd,dhe->bhte', h, Wk)
            v = jnp.einsum('btd,dhe->bhte', h, Wv)
            scores = jnp.einsum('bhqe,bhke->bhqk', q, k) * scale
            scores = jnp.where(mask[None, None], scores, -1000000000.0)
            p = _softmax(scores, axis=-1)
            o = jnp.einsum('bhqk,bhke->bhqe', p, v)
            o = jnp.einsum('bhte,hed->btd', o, Wo)
            mem = o[:, :M, :].copy()
            outs.append(o[:, M:, :])
        return jnp.concatenate(outs, axis=1)

    def _B_ref(x, w_gate, w_up, w_down):
        g = _silu(x @ w_gate)
        u = x @ w_up
        return g * u @ w_down
    x = A_x
    h = x + _A_ref(_layernorm(x, axis=-1), A_mem0, A_Wq, A_Wk, A_Wv, A_Wo, A_seg_len)
    h2 = h + _B_ref(_layernorm(h, axis=-1), B_w_gate, B_w_up, B_w_down)
    return h2
```

```python
import functools

import jax
import jax.numpy as jnp
import jax.experimental.pallas as pl
import jax.experimental.pallas.tpu as pltpu

F32 = jnp.float32
BF16 = jnp.bfloat16
U32 = jnp.uint32

S = 2048
D = 640
H = 32
DH = 192
M = 8
SEG = 32
NSEG = S // SEG
FF = 1536
NP = H // 2
PW = 2 * DH
QKVW = 3 * PW
P0 = 512
G = 24
RQ = 544
RO = 768
NSLOT = 3
KP = 48
TB = 256
EPS = 1e-5


def _ln(x):
    m = jnp.mean(x, axis=-1, keepdims=True)
    xc = x - m
    v = jnp.mean(xc * xc, axis=-1, keepdims=True)
    return xc / jnp.sqrt(v + EPS)


def _dot(a, b):
    return jnp.dot(a, b, preferred_element_type=F32)


def _dot_nt(a, b):
    return jax.lax.dot_general(a, b, (((1,), (1,)), ((), ())),
                               preferred_element_type=F32)


def _blockdiag(z):
    z32 = pltpu.bitcast(z, U32)
    lane = jax.lax.broadcasted_iota(jnp.int32, (KP // 2, 128), 1)
    mid = z32[:, 128:256]
    zero = jnp.zeros((KP // 2, 128), U32)
    top = jnp.concatenate([z32[:, :128], jnp.where(lane < 64, mid, zero), zero], axis=1)
    bot = jnp.concatenate([zero, jnp.where(lane >= 64, mid, zero), z32[:, 256:]], axis=1)
    return pltpu.bitcast(jnp.concatenate([top, bot], axis=0), BF16)


def _kernel(x_hbm, mem_hbm, wq_hbm, wk_hbm, wv_hbm, wo_hbm, wg_hbm, wu_hbm, wd_hbm,
            out_hbm,
            x_s, xn_s, mem_s, stage, w32, wo32, ring, obuf, lo_s, wg_s, wu_s, wd_s, out_s,
            sem_x, sem_w, sem_f, sem_o):
    w_hbms = (wq_hbm, wk_hbm, wv_hbm, wo_hbm)

    def w_copy(j, slot, m):
        return pltpu.make_async_copy(
            w_hbms[m].at[pl.ds(pl.multiple_of(j * PW, PW), PW)], stage.at[slot, m], sem_w.at[slot, m])

    x0_copy = pltpu.make_async_copy(x_hbm.at[pl.ds(0, P0)], x_s.at[pl.ds(G, P0)], sem_x.at[0])
    x1_copy = pltpu.make_async_copy(x_hbm.at[pl.ds(P0, S - P0)], x_s.at[pl.ds(G + P0, S - P0)], sem_x.at[1])
    mem_copy = pltpu.make_async_copy(mem_hbm, mem_s, sem_x.at[2])
    f_copies = [pltpu.make_async_copy(src, dst, sem_f.at[i])
                for i, (src, dst) in enumerate(((wg_hbm, wg_s), (wu_hbm, wu_s), (wd_hbm, wd_s)))]

    x0_copy.start()
    for m in range(4):
        w_copy(0, 0, m).start()
    x1_copy.start()
    mem_copy.start()
    for m in range(4):
        w_copy(1, 1, m).start()

    x0_copy.wait()
    for r in range(0, P0, 128):
        xn_s[r:r + 128, :] = _ln(x_s[G + r:G + r + 128, :].astype(F32)).astype(BF16)
    x1_copy.wait()
    mem_copy.wait()

    LNR = (S - P0) // NP

    def prologue(j, carry):
        slot = j % NSLOT

        @pl.when(j + 2 < NP)
        def _():
            for m in range(4):
                w_copy(j + 2, (j + 2) % NSLOT, m).start()

        for m in range(4):
            w_copy(j, slot, m).wait()
        for m in range(3):
            wt = stage[slot, m]
            col = pl.multiple_of(j * QKVW + m * PW, 128)
            ring[0:P0, pl.ds(col, PW)] = _dot_nt(xn_s[0:P0, :], wt).astype(BF16)
            w32[:, pl.ds(col, PW)] = pltpu.bitcast(wt.T, U32)
        wo32[pl.ds(pl.multiple_of(j * (PW // 2), PW // 2), PW // 2), :] = pltpu.bitcast(stage[slot, 3], U32)
        r = pl.multiple_of(P0 + j * LNR, 16)
        xn_s[pl.ds(r, LNR), :] = _ln(x_s[pl.ds(pl.multiple_of(G + r, 8), LNR), :].astype(F32)).astype(BF16)
        return carry

    jax.lax.fori_loop(0, NP, prologue, 0)

    for c in f_copies:
        c.start()

    row = jax.lax.broadcasted_iota(jnp.int32, (KP, 2 * KP), 0)
    col = jax.lax.broadcasted_iota(jnp.int32, (KP, 2 * KP), 1)
    is_a = col < KP
    kcol = jnp.where(is_a, col, col - KP)
    is_key = kcol < SEG + M
    visible = (row >= SEG) | (kcol >= SEG) | (kcol <= row)
    scale = DH ** -0.5
    neg_inf = float("-inf")

    def step(s, mem):
        t0 = pl.multiple_of(P0 + G * s, 8)
        lhs = jnp.concatenate([xn_s[pl.ds(t0, G), :], mem], axis=0)
        wr = [pl.multiple_of(((P0 + G * s) // 8 + g) % (RQ // 8) * 8, 8) for g in range(G // 8)]
        rr = pl.multiple_of((SEG * s) % RQ, SEG)
        ow = pl.multiple_of((SEG * s + G) % RO, 8)
        orr = pl.multiple_of((G * s) % RO, 8)
        lo_s[0:G, :] = obuf[pl.ds(orr, G), :]
        mz, p = {}, {}

        def stage_a(j):
            c0 = j * QKVW
            qkv = _dot(lhs, pltpu.bitcast(w32[:, c0:c0 + QKVW], BF16))
            for g in range(G // 8):
                ring[pl.ds(wr[g], 8), c0:c0 + QKVW] = qkv[8 * g:8 * g + 8].astype(BF16)
            mz[j] = jnp.concatenate([qkv[G:], jnp.zeros((8, QKVW), F32)], axis=0).astype(BF16)

        def tok(j, m):
            c = j * QKVW + m * PW
            return ring[pl.ds(rr, SEG), c:c + PW]

        def rows(t, j, m):
            return jnp.concatenate([t, mz[j][:, m * PW:(m + 1) * PW]], axis=0)

        def stage_b(j, qt, kt):
            sc = _dot_nt(rows(qt, j, 0), _blockdiag(rows(kt, j, 1))) * scale
            sc = jnp.where(visible, sc, -1e9)
            sc = jnp.where(is_key, sc, neg_inf)
            ma = jnp.max(jnp.where(is_a, sc, neg_inf), axis=1, keepdims=True)
            mb = jnp.max(jnp.where(is_a, neg_inf, sc), axis=1, keepdims=True)
            e = jnp.exp(sc - jnp.where(is_a, ma, mb))
            sa = jnp.sum(jnp.where(is_a, e, 0.0), axis=1, keepdims=True)
            sb = jnp.sum(jnp.where(is_a, 0.0, e), axis=1, keepdims=True)
            p[j] = (e * jnp.where(is_a, 1.0 / sa, 1.0 / sb)).astype(BF16)

        def stage_c(j, vt):
            o = _dot(p[j], _blockdiag(rows(vt, j, 2)))
            for g in range(SEG // 8):
                og = pl.multiple_of(((SEG * s + G) // 8 + g) % (RO // 8) * 8, 8)
                obuf[pl.ds(og, 8), j * PW:(j + 1) * PW] = o[8 * g:8 * g + 8].astype(BF16)
            lo_s[G:G + M, j * PW:(j + 1) * PW] = o[SEG:SEG + M].astype(BF16)

        def stage_d(j, acc):
            d = _dot(lo_s[:, j * PW:(j + 1) * PW],
                     pltpu.bitcast(wo32[j * (PW // 2):(j + 1) * (PW // 2), :], BF16))
            return d if acc is None else acc + d

        for t in range(NP):
            if t >= 1:
                qt, kt = tok(t - 1, 0), tok(t - 1, 1)
            if t >= 2:
                vt = tok(t - 2, 2)
            stage_a(t)
            if t >= 1:
                stage_b(t - 1, qt, kt)
            if t >= 2:
                stage_c(t - 2, vt)
        acc = stage_d(0, None)
        stage_b(NP - 1, tok(NP - 1, 0), tok(NP - 1, 1))
        acc = stage_d(1, acc)
        acc = stage_d(2, acc)
        stage_c(NP - 2, tok(NP - 2, 2))
        for j in range(3, 8):
            acc = stage_d(j, acc)
        stage_c(NP - 1, tok(NP - 1, 2))
        for j in range(8, NP):
            acc = stage_d(j, acc)
        h0 = pl.multiple_of(G * s, 8)
        x_s[pl.ds(h0, G), :] = (x_s[pl.ds(h0, G), :].astype(F32) + acc[:G]).astype(BF16)
        return acc[G:].astype(BF16)

    obuf[0:G, :] = jnp.zeros((G, H * DH), BF16)
    x_s[0:G, :] = jnp.zeros((G, D), BF16)
    jax.lax.fori_loop(0, NSEG, step, mem_s[...])

    L0 = G * NSEG
    LB = (S + G - L0) // 2
    for r in range(L0, S + G, LB):
        a = _dot(obuf[r % RO:r % RO + LB, :], pltpu.bitcast(wo32[...], BF16))
        x_s[r:r + LB, :] = (x_s[r:r + LB, :].astype(F32) + a).astype(BF16)

    for c in f_copies:
        c.wait()

    def o_copy(i, slot):
        return pltpu.make_async_copy(
            out_s.at[slot], out_hbm.at[pl.ds(pl.multiple_of(i * TB, TB), TB)], sem_o.at[slot])

    def ffn(i, carry):
        slot = i % 2

        @pl.when(i >= 2)
        def _():
            o_copy(i - 2, slot).wait()

        r = pl.multiple_of(i * TB, TB)
        h = x_s[pl.ds(pl.multiple_of(G + r, 8), TB), :].astype(F32)
        hn = _ln(h).astype(BF16)
        g = _dot(hn, wg_s[...])
        u = _dot(hn, wu_s[...])
        a = (g * jax.nn.sigmoid(g) * u).astype(BF16)
        out_s[slot] = (h + _dot(a, wd_s[...])).astype(BF16)
        o_copy(i, slot).start()
        return carry

    nblk = S // TB
    jax.lax.fori_loop(0, nblk, ffn, 0)
    o_copy(nblk - 2, (nblk - 2) % 2).wait()
    o_copy(nblk - 1, (nblk - 1) % 2).wait()


@functools.partial(jax.jit, static_argnames=("A_seg_len",))
def pallas_sequential_preLN__memory_aug_recurrent_mem_tr__swiglu_ffn__prompt_kernel(
    A_x: jax.Array,
    A_mem0: jax.Array,
    A_Wq: jax.Array,
    A_Wk: jax.Array,
    A_Wv: jax.Array,
    A_Wo: jax.Array,
    A_seg_len,
    B_x: jax.Array,
    B_w_gate: jax.Array,
    B_w_up: jax.Array,
    B_w_down: jax.Array,
):
    assert A_x.shape == (1, S, D) and A_Wq.shape == (D, H, DH) and A_seg_len == SEG
    x = A_x.reshape(S, D)
    mem0 = A_mem0.reshape(M, D)
    wq_t = A_Wq.transpose(1, 2, 0).reshape(H * DH, D)
    wk_t = A_Wk.transpose(1, 2, 0).reshape(H * DH, D)
    wv_t = A_Wv.transpose(1, 2, 0).reshape(H * DH, D)
    wo = A_Wo.reshape(H * DH, D)

    any_spec = pl.BlockSpec(memory_space=pl.ANY)
    out = pl.pallas_call(
        _kernel,
        in_specs=[any_spec] * 9,
        out_specs=any_spec,
        out_shape=jax.ShapeDtypeStruct((S, D), BF16),
        scratch_shapes=[
            pltpu.VMEM((S + G, D), BF16),
            pltpu.VMEM((S, D), BF16),
            pltpu.VMEM((M, D), BF16),
            pltpu.VMEM((NSLOT, 4, PW, D), BF16),
            pltpu.VMEM((D // 2, NP * QKVW), U32),
            pltpu.VMEM((H * DH // 2, D), U32),
            pltpu.VMEM((RQ, NP * QKVW), BF16),
            pltpu.VMEM((RO, H * DH), BF16),
            pltpu.VMEM((G + M, H * DH), BF16),
            pltpu.VMEM((D, FF), BF16),
            pltpu.VMEM((D, FF), BF16),
            pltpu.VMEM((FF, D), BF16),
            pltpu.VMEM((2, TB, D), BF16),
            pltpu.SemaphoreType.DMA((3,)),
            pltpu.SemaphoreType.DMA((NSLOT, 4)),
            pltpu.SemaphoreType.DMA((3,)),
            pltpu.SemaphoreType.DMA((2,)),
        ],
        compiler_params=pltpu.CompilerParams(vmem_limit_bytes=120 * 1024 * 1024),
    )(x, mem0, wq_t, wk_t, wv_t, wo, B_w_gate, B_w_up, B_w_down)
    return out.reshape(1, S, D)
```

```python
import functools

import jax
import jax.numpy as jnp
import jax.experimental.pallas as pl
import jax.experimental.pallas.tpu as pltpu

F32 = jnp.float32
BF16 = jnp.bfloat16
U32 = jnp.uint32

S = 2048
D = 640
H = 32
DH = 192
M = 8
SEG = 32
NSEG = S // SEG
NIT = NSEG // 2
FF = 1536
NP = H // 2
PW = 2 * DH
QKVW = 3 * PW
DQ = 8
P0 = NSEG * DQ
PPI = 2
PM = 128
KPA, KPB = 48, 64
FB = 2 * SEG
FC = 512
OUT_SPLIT = (0, 28 * FB, S - FB, S)
EPS = 1e-5
LN_AT = 6
LAG_A = 3
LAG_B = 2
UP_A = tuple(range(1, 16))
UP_B = (1, 2, 3)
DOWN_B = (14, 15, ("d", 15))
EARLY_D = 10
D_FROM = 4
TAIL_A = (2, 2, 5, 9)
TAIL_B = (11, 12, 14)


def _ln(x):
    m = jnp.mean(x, axis=-1, keepdims=True)
    xc = x - m
    v = jnp.mean(xc * xc, axis=-1, keepdims=True)
    return xc / jnp.sqrt(v + EPS)


def _dot(a, b):
    return jnp.dot(a, b, preferred_element_type=F32)


def _dot_nt(a, b):
    return jax.lax.dot_general(a, b, (((1,), (1,)), ((), ())),
                               preferred_element_type=F32)


def _bf(w32):
    return pltpu.bitcast(w32, BF16)


def _pk(x):
    return pltpu.bitcast(x.astype(BF16), U32)


def _halves(lo, hi):
    sub = jax.lax.broadcasted_iota(jnp.int32, lo.shape, 0)
    return jnp.where(sub < 4, lo, hi)


def _blockdiag(z32):
    n = z32.shape[0]
    lane = jax.lax.broadcasted_iota(jnp.int32, (n, 128), 1)
    mid = z32[:, 128:256]
    zero = jnp.zeros((n, 128), U32)
    top = jnp.concatenate([z32[:, :128], jnp.where(lane < 64, mid, zero), zero], axis=1)
    bot = jnp.concatenate([zero, jnp.where(lane >= 64, mid, zero), z32[:, 256:]], axis=1)
    return _bf(jnp.concatenate([top, bot], axis=0))


def _masks(odd):
    nq, kp = (SEG + M + DQ, KPB) if odd else (SEG - DQ + M, KPA)
    row = jax.lax.broadcasted_iota(jnp.int32, (nq, 2 * kp), 0)
    col = jax.lax.broadcasted_iota(jnp.int32, (nq, 2 * kp), 1)
    is_a = col < kp
    kc = jnp.where(is_a, col, col - kp)

    def pos(i):
        return jnp.where(i < 16, i + 16, jnp.where(i < 32, i - 16, i & 7))

    def between(i, lo, hi):
        return (i >= lo) & (i < hi)

    visible = between(kc, 16, 24) | (kc >= 48) | between(row, 16, 24) | (pos(kc) <= pos(row))
    if odd:
        prev_q = between(row, 32, 40)
        prev_k = between(kc, 32, 40) | between(kc, 48, 56)
        own_k = (kc < 32) | between(kc, 40, 48)
        is_key = (prev_q & prev_k) | (~prev_q & own_k)
    else:
        is_key = kc < 40
    return is_a, is_key, visible


def _kernel(x_hbm, x3_hbm, mem_hbm, wq_hbm, wk_hbm, wv_hbm, wo_hbm, wg_hbm, wu_hbm, wd_hbm,
            out_hbm,
            x_s, xl_s, xn_s, mem_s, stage, w32, wo32, wg32, wu32, wd32, pool,
            lo_s, mkv_s, hn_s, act_s,
            sem, sem_o):
    w_hbms = (wq_hbm, wk_hbm, wv_hbm)

    def w_copy(j, m, n=1):
        rows = pl.ds(pl.multiple_of(j * PW, PW), n * PW)
        return pltpu.make_async_copy(w_hbms[m].at[rows], stage.at[m, rows], sem.at[8 + 3 * j + m])

    x0_copy = pltpu.make_async_copy(x3_hbm.at[:, pl.ds(0, DQ), :], xl_s, sem.at[0])
    x1_copy = pltpu.make_async_copy(x_hbm, x_s, sem.at[1])
    mem_copy = pltpu.make_async_copy(mem_hbm, mem_s, sem.at[2])
    wo_copy = pltpu.make_async_copy(wo_hbm.bitcast(U32), wo32, sem.at[3])
    f_copies = [pltpu.make_async_copy(src.bitcast(U32), dst, sem.at[4 + i])
                for i, (src, dst) in enumerate(((wg_hbm, wg32), (wu_hbm, wu32), (wd_hbm, wd32)))]

    x0_copy.start()
    for j in (0, 1):
        for m in range(3):
            w_copy(j, m).start()
    for j in range(2, NP, PPI):
        for m in range(3):
            w_copy(j, m, PPI).start()
        if j == 2:
            x1_copy.start()
            mem_copy.start()

    x0_copy.wait()
    for g in range(0, NSEG, 16):
        xl = xl_s[g:g + 16].astype(F32).reshape(128, D)
        xn_s[4 * g:4 * g + 64, :] = _pk(_ln(xl))

    def ln_next(t):
        xn = _pk(_ln(x_s[pl.ds(pl.multiple_of(t, FB), FB), :].astype(F32)))
        pool[NIT:NIT + 4, :, 0:D] = xn.reshape(4, 8, D)

    def project(j, m):
        wt = stage[m, pl.ds(pl.multiple_of(j * PW, PW), PW), :]
        col = pl.ds(pl.multiple_of(j * QKVW + m * PW, 128), PW)
        for r in range(0, P0, PM):
            y = _dot_nt(_bf(xn_s[r // 2:(r + PM) // 2, :]), wt)
            pool[r // 16:(r + PM) // 16, :, col] = _pk(y).reshape(PM // 16, 8, PW)
        w32[:, col] = pltpu.bitcast(wt.T, U32)

    for m in range(3):
        w_copy(0, m).wait()
        project(0, m)
    for m in range(3):
        w_copy(1, m).wait()
    for m in range(3):
        project(1, m)
    wo_copy.start()
    for c in f_copies:
        c.start()

    def prologue(i, carry):
        for m in range(3):
            w_copy(2 + PPI * i, m, PPI).wait()
        for jj in range(PPI):
            for m in range(3):
                project(2 + PPI * i + jj, m)
        return carry

    jax.lax.fori_loop(0, (NP - 2) // PPI, prologue, 0)
    x1_copy.wait()
    mem_copy.wait()
    wo_copy.wait()
    ln_next(0)

    scale = DH ** -0.5
    neg_inf = float("-inf")

    def step(xn_lo, xn_hi, mem, u, odd, fillers):
        mem_pk = _pk(jnp.concatenate([mem, jnp.zeros((8, D), F32)], axis=0))
        lhs = _bf(jnp.concatenate([xn_hi, _halves(mem_pk, xn_lo)], axis=0))
        nq = SEG + M + DQ if odd else SEG - DQ + M
        is_a, is_key, visible = _masks(odd)
        cur, p = {}, {}

        def stage_a(j):
            cur[j] = _pk(_dot(lhs, _bf(w32[:, j * QKVW:(j + 1) * QKVW])))
            if not odd:
                mkv_s[:, 2 * PW * j:2 * PW * (j + 1)] = _halves(
                    cur[j][8:16, PW:], jnp.zeros((8, 2 * PW), U32))

        def tok(j, m):
            if m == 0 and not odd:
                return None
            return pool[u, :, j * QKVW + m * PW:j * QKVW + (m + 1) * PW]

        def rows(lead, j, m):
            parts = [cur[j][:, m * PW:(m + 1) * PW]]
            if odd:
                parts.append(lead)
                if m:
                    parts.append(mkv_s[:, 2 * PW * j + (m - 1) * PW:2 * PW * j + m * PW])
            elif m:
                parts.append(_halves(lead, jnp.zeros((8, PW), U32)))
            return jnp.concatenate(parts, axis=0)

        def stage_b(j, qt, kt):
            sc = _dot_nt(_bf(rows(qt, j, 0)), _blockdiag(rows(kt, j, 1))) * scale
            sc = jnp.where(visible, sc, -1e9)
            sc = jnp.where(is_key, sc, neg_inf)
            ma = jnp.max(jnp.where(is_a, sc, neg_inf), axis=1, keepdims=True)
            mb = jnp.max(jnp.where(is_a, neg_inf, sc), axis=1, keepdims=True)
            e = jnp.exp(sc - jnp.where(is_a, ma, mb))
            sa = jnp.sum(jnp.where(is_a, e, 0.0), axis=1, keepdims=True)
            sb = jnp.sum(jnp.where(is_a, 0.0, e), axis=1, keepdims=True)
            p[j] = (e * jnp.where(is_a, 1.0 / sa, 1.0 / sb)).astype(BF16)

        def stage_c(j, vt):
            o = _dot(p[j], _blockdiag(rows(vt, j, 2)))
            lo_s[0:nq // 2, j * PW:(j + 1) * PW] = _pk(o)

        def stage_d(j, acc):
            d = _dot(_bf(lo_s[0:nq // 2, j * PW:(j + 1) * PW]),
                     _bf(wo32[j * (PW // 2):(j + 1) * (PW // 2), :]))
            return d if acc is None else acc + d

        def fill(key):
            for f in fillers.get(key, ()):
                f()

        acc, nd = None, 0
        lag = LAG_B if odd else LAG_A
        for t in range(NP):
            if t >= 1:
                qt, kt = tok(t - 1, 0), tok(t - 1, 1)
            if t >= lag:
                vt = tok(t - lag, 2)
            stage_a(t)
            fill(t)
            if odd and t >= D_FROM and nd < EARLY_D:
                acc = stage_d(nd, acc)
                nd += 1
            if t >= 1:
                stage_b(t - 1, qt, kt)
            if t >= lag:
                stage_c(t - lag, vt)
        tail = TAIL_B if odd else TAIL_A
        for j in range(nd, NP):
            if j == tail[0]:
                stage_b(NP - 1, tok(NP - 1, 0), tok(NP - 1, 1))
            for i in range(lag):
                if j == tail[1 + i]:
                    stage_c(NP - lag + i, tok(NP - lag + i, 2))
            fill(("d", j))
            acc = stage_d(j, acc)

        def residual(t, a):
            hr = pl.ds(pl.multiple_of(t, 8), a.shape[0])
            x_s[hr, :] = (x_s[hr, :].astype(F32) + a).astype(BF16)

        t0 = FB * u + SEG if odd else FB * u
        residual(t0 + 16, acc[0:16])
        residual(t0 + 8, acc[24:32])
        if odd:
            residual(t0 - SEG, acc[32:40])
            residual(t0, acc[40:48])
        return acc[16:24]

    def ffn_ln(r):
        hn_s[...] = _pk(_ln(x_s[pl.ds(r, FB), :].astype(F32)))

    gate = {}

    def ffn_gate(c, w):
        g = _dot(_bf(hn_s[...]), _bf(wg32[:, c:c + w]))
        gate[c] = g * jax.nn.sigmoid(g)

    def ffn_up(c, w):
        u = _dot(_bf(hn_s[...]), _bf(wu32[:, c:c + w]))
        act_s[:, c:c + w] = _pk(gate.pop(c) * u)

    def ffn_down(r, c, w):
        y = _dot(_bf(act_s[...]), _bf(wd32[:, c:c + w]))
        x_s[pl.ds(r, FB), c:c + w] = (x_s[pl.ds(r, FB), c:c + w].astype(F32) + y).astype(BF16)

    def out_copy(i):
        r = pl.ds(OUT_SPLIT[i], OUT_SPLIT[i + 1] - OUT_SPLIT[i])
        return pltpu.make_async_copy(x_s.at[r], out_hbm.at[r], sem_o.at[i])

    def iteration(u, mem, with_ffn):
        fill_a, fill_b, mid, end = {}, {}, [], []
        if with_ffn:
            @pl.when(u == OUT_SPLIT[1] // FB + 1)
            def _():
                out_copy(0).start()

            fr = pl.multiple_of(FB * u - FB, FB)
            ffn_ln(fr)
            ups = [functools.partial(f, c, 128) for c in range(0, FF, 128) for f in (ffn_gate, ffn_up)]
            downs = [functools.partial(ffn_down, fr, c, 128) for c in range(0, D, 128)]
            for t in UP_A:
                fill_a.setdefault(t, []).append(ups.pop(0))
            mid = [ups.pop(0) for _ in range(len(ups) - len(UP_B))]
            for t in UP_B:
                fill_b.setdefault(t, []).append(ups.pop(0))
            for t in DOWN_B:
                fill_b.setdefault(t, []).append(downs.pop(0))
            end = downs
        xn = [pool[NIT + i, :, 0:D] for i in range(4)]
        fill_a.setdefault(LN_AT, []).append(lambda: ln_next(jnp.minimum(FB * (u + 1), S - FB)))
        mem = step(xn[0], xn[1], mem, u, False, fill_a)
        for f in mid:
            f()
        mem = step(xn[2], xn[3], mem, u, True, fill_b)
        for f in end:
            f()
        return mem

    carry = iteration(0, mem_s[...].astype(F32), False)
    for c in f_copies:
        c.wait()
    jax.lax.fori_loop(1, NIT, functools.partial(iteration, with_ffn=True), carry)

    out_copy(1).start()
    ffn_ln(S - FB)
    for c in range(0, FF, FC):
        ffn_gate(c, FC)
        ffn_up(c, FC)
    ffn_down(S - FB, 0, D)
    out_copy(2).start()
    for i in range(3):
        out_copy(i).wait()


@jax.jit
def pallas_sequential_preLN__memory_aug_recurrent_mem_tr__swiglu_ffn__prompt_kernel(
    A_x: jax.Array,
    A_mem0: jax.Array,
    A_Wq: jax.Array,
    A_Wk: jax.Array,
    A_Wv: jax.Array,
    A_Wo: jax.Array,
    A_seg_len: jax.Array,
    B_x: jax.Array,
    B_w_gate: jax.Array,
    B_w_up: jax.Array,
    B_w_down: jax.Array,
):
    assert A_x.shape == (1, S, D) and A_Wq.shape == (D, H, DH) and A_mem0.shape == (1, M, D)
    x = A_x.reshape(S, D)
    mem0 = A_mem0.reshape(M, D)
    wq_t = A_Wq.transpose(1, 2, 0).reshape(H * DH, D)
    wk_t = A_Wk.transpose(1, 2, 0).reshape(H * DH, D)
    wv_t = A_Wv.transpose(1, 2, 0).reshape(H * DH, D)
    wo = A_Wo.reshape(H * DH, D)

    any_spec = pl.BlockSpec(memory_space=pl.ANY)
    out = pl.pallas_call(
        _kernel,
        in_specs=[any_spec] * 10,
        out_specs=any_spec,
        out_shape=jax.ShapeDtypeStruct((S, D), BF16),
        scratch_shapes=[
            pltpu.VMEM((S, D), BF16),
            pltpu.VMEM((NSEG, DQ, D), BF16),
            pltpu.VMEM((P0 // 2, D), U32),
            pltpu.VMEM((M, D), BF16),
            pltpu.VMEM((3, H * DH, D), BF16),
            pltpu.VMEM((D // 2, NP * QKVW), U32),
            pltpu.VMEM((H * DH // 2, D), U32),
            pltpu.VMEM((D // 2, FF), U32),
            pltpu.VMEM((D // 2, FF), U32),
            pltpu.VMEM((FF // 2, D), U32),
            pltpu.VMEM((NIT + 4, 8, NP * QKVW), U32),
            pltpu.VMEM(((SEG + M + DQ) // 2, H * DH), U32),
            pltpu.VMEM((8, 2 * H * DH), U32),
            pltpu.VMEM((FB // 2, D), U32),
            pltpu.VMEM((FB // 2, FF), U32),
            pltpu.SemaphoreType.DMA((8 + 3 * NP,)),
            pltpu.SemaphoreType.DMA((3,)),
        ],
        compiler_params=pltpu.CompilerParams(vmem_limit_bytes=120 * 1024 * 1024),
    )(x, x.reshape(NSEG, SEG, D), mem0, wq_t, wk_t, wv_t, wo, B_w_gate, B_w_up, B_w_down)
    return out.reshape(1, S, D)
```

```python
import functools

import jax
import jax.numpy as jnp
import jax.experimental.pallas as pl
import jax.experimental.pallas.tpu as pltpu

F32 = jnp.float32
BF16 = jnp.bfloat16
U32 = jnp.uint32

S = 2048
D = 640
H = 32
DH = 192
M = 8
SEG = 32
NSEG = S // SEG
NIT = NSEG // 2
FF = 1536
NP = H // 2
PW = 2 * DH
QKVW = 3 * PW
DQ = 8
P0 = NSEG * DQ
PPI = 2
NPI = (NP - 2) // PPI
PM = 128
KPA, KPB = 48, 64
FB = 2 * SEG
FC = 512
OUT_SPLIT = (0, 28 * FB, S - FB, S)
EPS = 1e-5
LOG2E = 1.4426950408889634
LN_AT = 5
LAG_A = 3
LAG_B = 2
UP_A = tuple(range(1, 16)) + (("d", 2),)
UP_B = (1, 2, 3, 4, 5)
DOWN_B = (14, 15, ("d", 15))
EARLY_D = 10
D_FROM = 4
TAIL_A = (2, 2, 5, 9)
TAIL_B = (11, 12, 14)


def _ln(x):
    m = jnp.mean(x, axis=-1, keepdims=True)
    xc = x - m
    v = jnp.mean(xc * xc, axis=-1, keepdims=True)
    return xc * jax.lax.rsqrt(v + EPS)


def _dot(a, b):
    return jnp.dot(a, b, preferred_element_type=F32)


def _dot_nt(a, b):
    return jax.lax.dot_general(a, b, (((1,), (1,)), ((), ())),
                               preferred_element_type=F32)


def _bf(w32):
    return pltpu.bitcast(w32, BF16)


def _pk(x):
    return pltpu.bitcast(x.astype(BF16), U32)


def _halves(lo, hi):
    sub = jax.lax.broadcasted_iota(jnp.int32, lo.shape, 0)
    return jnp.where(sub < 4, lo, hi)


def _blockdiag(z32):
    n = z32.shape[0]
    lane = jax.lax.broadcasted_iota(jnp.int32, (n, 128), 1)
    mid = z32[:, 128:256]
    zero = jnp.zeros((n, 128), U32)
    top = jnp.concatenate([z32[:, :128], jnp.where(lane < 64, mid, zero), zero], axis=1)
    bot = jnp.concatenate([zero, jnp.where(lane >= 64, mid, zero), z32[:, 256:]], axis=1)
    return _bf(jnp.concatenate([top, bot], axis=0))


def _masks(odd):
    nq, kp = (SEG + M + DQ, KPB) if odd else (SEG - DQ + M, KPA)
    row = jax.lax.broadcasted_iota(jnp.int32, (nq, 128), 0)
    col = jax.lax.broadcasted_iota(jnp.int32, (nq, 128), 1)
    is_a = col < kp
    kc = jnp.where(is_a, col, col - kp)

    def pos(i):
        return jnp.where(i < 16, i + 16, jnp.where(i < 32, i - 16, i & 7))

    def between(i, lo, hi):
        return (i >= lo) & (i < hi)

    visible = between(kc, 16, 24) | (kc >= 48) | between(row, 16, 24) | (pos(kc) <= pos(row))
    if odd:
        prev_q = between(row, 32, 40)
        prev_k = between(kc, 32, 40) | between(kc, 48, 56)
        own_k = (kc < 32) | between(kc, 40, 48)
        is_key = (prev_q & prev_k) | (~prev_q & own_k)
    else:
        is_key = kc < 40
    return is_a, is_key, visible


def _kernel(x_hbm, x3_hbm, mem_hbm, wq_hbm, wk_hbm, wv_hbm, wo_hbm, wg_hbm, wu_hbm, wd_hbm,
            out_hbm,
            x_s, xl_s, xn_s, mem_s, stage, w32, wo32, wg32, wu32, wd32, pool,
            lo_s, cur_s, hn_s, act_s,
            sem, sem_o):
    w_hbms = (wq_hbm, wk_hbm, wv_hbm)

    def w_copy(j, m, n, k):
        rows = pl.ds(pl.multiple_of(j * PW, PW), n * PW)
        return pltpu.make_async_copy(w_hbms[m].at[rows], stage.at[m, rows], sem.at[k])

    x0_copy = pltpu.make_async_copy(x3_hbm.at[:, pl.ds(0, DQ), :], xl_s, sem.at[0])
    q0_copy = w_copy(0, 0, 1, 1)
    kv0_copies = [w_copy(0, m, 1, 2) for m in (1, 2)]
    p1_copies = [w_copy(1, m, 1, 3) for m in range(3)] + [
        pltpu.make_async_copy(x_hbm.at[pl.ds(0, FB)], x_s.at[pl.ds(0, FB)], sem.at[3])]
    x1_copy = pltpu.make_async_copy(x_hbm.at[pl.ds(FB, S - FB)], x_s.at[pl.ds(FB, S - FB)], sem.at[4])
    mem_copy = pltpu.make_async_copy(mem_hbm, mem_s, sem.at[4])
    wo_copy = pltpu.make_async_copy(wo_hbm.bitcast(U32), wo32, sem.at[4])
    f_copies = [pltpu.make_async_copy(src.bitcast(U32), dst, sem.at[5])
                for src, dst in ((wg_hbm, wg32), (wu_hbm, wu32), (wd_hbm, wd32))]

    def group_copies(i):
        return [w_copy(2 + PPI * i, m, PPI, 6 + i) for m in range(3)]

    for c in [x0_copy, q0_copy] + kv0_copies + p1_copies:
        c.start()
    for i in range(NPI):
        for c in group_copies(i):
            c.start()
        if i == 0:
            x1_copy.start()
            mem_copy.start()

    x0_copy.wait()
    for g in range(0, NSEG, 16):
        xl = xl_s[g:g + 16].astype(F32).reshape(128, D)
        xn_s[4 * g:4 * g + 64, :] = _pk(_ln(xl))

    def ln_next(t):
        xn = _pk(_ln(x_s[pl.ds(pl.multiple_of(t, FB), FB), :].astype(F32)))
        pool[NIT:NIT + 4, :, 0:D] = xn.reshape(4, 8, D)

    def chunk(j, m):
        wt = stage[m, pl.ds(pl.multiple_of(j * PW, PW), PW), :]
        col = pl.ds(pl.multiple_of(j * QKVW + m * PW, 128), PW)
        for r in range(0, P0, PM):
            y = _dot_nt(_bf(xn_s[r // 2:(r + PM) // 2, :]), wt)
            pool[r // 16:(r + PM) // 16, :, col] = _pk(y).reshape(PM // 16, 8, PW)
        w32[:, col] = pltpu.bitcast(wt.T, U32)

    q0_copy.wait()
    chunk(0, 0)
    for c in kv0_copies:
        c.wait()
    chunk(0, 1)
    chunk(0, 2)
    for c in p1_copies:
        c.wait()
    ln_next(0)
    for m in range(3):
        chunk(1, m)
    wo_copy.start()
    for c in f_copies:
        c.start()

    def prologue(i, carry):
        for c in group_copies(i):
            c.wait()
        for jj in range(PPI):
            for m in range(3):
                chunk(2 + PPI * i + jj, m)
        return carry

    jax.lax.fori_loop(0, NPI, prologue, 0)
    x1_copy.wait()
    mem_copy.wait()
    wo_copy.wait()

    scale = DH ** -0.5
    neg_inf = float("-inf")

    def step(xn_lo, xn_hi, mem, u, odd, fillers):
        mem_pk = _pk(jnp.concatenate([mem, jnp.zeros((8, D), F32)], axis=0))
        lhs = _bf(jnp.concatenate([xn_hi, _halves(mem_pk, xn_lo)], axis=0))
        nq = SEG + M + DQ if odd else SEG - DQ + M
        is_a, is_key, visible = _masks(odd)
        p = {}

        def stage_a(j):
            cs = slice(j * QKVW, (j + 1) * QKVW)
            cur_s[int(odd), :, cs] = _pk(_dot(lhs, _bf(w32[:, cs])))

        def tok(j, m):
            if m == 0 and not odd:
                return None
            return pool[u, :, j * QKVW + m * PW:j * QKVW + (m + 1) * PW]

        def rows(lead, j, m):
            cs = slice(j * QKVW + m * PW, j * QKVW + (m + 1) * PW)
            zero = jnp.zeros((8, PW), U32)
            parts = [cur_s[int(odd), :, cs]]
            if odd:
                parts.append(lead)
                if m:
                    parts.append(_halves(cur_s[0, 8:16, cs], zero))
            elif m:
                parts.append(_halves(lead, zero))
            return jnp.concatenate(parts, axis=0)

        def stage_b(j, qt, kt):
            sc = _dot_nt(_bf(rows(qt, j, 0)), _blockdiag(rows(kt, j, 1)))
            sc = sc * (scale * LOG2E)
            nk = sc.shape[1]
            if nk < 128:
                sc = jnp.concatenate([sc, jnp.full((nq, 128 - nk), neg_inf, F32)], axis=1)
            sc = jnp.where(visible, sc, -1e9 * LOG2E)
            sc = jnp.where(is_key, sc, neg_inf)
            ma = jnp.max(jnp.where(is_a, sc, neg_inf), axis=1, keepdims=True)
            mb = jnp.max(jnp.where(is_a, neg_inf, sc), axis=1, keepdims=True)
            e = jnp.exp2(sc - jnp.where(is_a, ma, mb))
            sa = jnp.sum(jnp.where(is_a, e, 0.0), axis=1, keepdims=True)
            sb = jnp.sum(jnp.where(is_a, 0.0, e), axis=1, keepdims=True)
            den = jnp.where(is_a, sa, sb)
            r = pl.reciprocal(den, approx=True)
            p[j] = (e * (r * (2.0 - den * r)))[:, 0:nk].astype(BF16)

        def stage_c(j, vt):
            o = _dot(p[j], _blockdiag(rows(vt, j, 2)))
            lo_s[0:nq // 2, j * PW:(j + 1) * PW] = _pk(o)

        def stage_d(j, acc):
            d = _dot(_bf(lo_s[0:nq // 2, j * PW:(j + 1) * PW]),
                     _bf(wo32[j * (PW // 2):(j + 1) * (PW // 2), :]))
            return d if acc is None else acc + d

        def fill(key):
            for f in fillers.get(key, ()):
                f()

        acc, nd = None, 0
        lag = LAG_B if odd else LAG_A
        for t in range(NP):
            if t >= 1:
                qt, kt = tok(t - 1, 0), tok(t - 1, 1)
            if t >= lag:
                vt = tok(t - lag, 2)
            stage_a(t)
            fill(t)
            if odd and t >= D_FROM and nd < EARLY_D:
                acc = stage_d(nd, acc)
                nd += 1
            if t >= 1:
                stage_b(t - 1, qt, kt)
            if t >= lag:
                stage_c(t - lag, vt)
        tail = TAIL_B if odd else TAIL_A
        for j in range(nd, NP):
            if j == tail[0]:
                stage_b(NP - 1, tok(NP - 1, 0), tok(NP - 1, 1))
            for i in range(lag):
                if j == tail[1 + i]:
                    stage_c(NP - lag + i, tok(NP - lag + i, 2))
            fill(("d", j))
            acc = stage_d(j, acc)

        def residual(t, a):
            hr = pl.ds(pl.multiple_of(t, 8), a.shape[0])
            x_s[hr, :] = (x_s[hr, :].astype(F32) + a).astype(BF16)

        t0 = FB * u + SEG if odd else FB * u
        residual(t0 + 16, acc[0:16])
        residual(t0 + 8, acc[24:32])
        if odd:
            residual(t0 - SEG, acc[32:40])
            residual(t0, acc[40:48])
        return acc[16:24]

    def ffn_ln(r):
        hn_s[...] = _pk(_ln(x_s[pl.ds(r, FB), :].astype(F32)))

    gate = {}

    def ffn_gate(c, w):
        g = _dot(_bf(hn_s[...]), _bf(wg32[:, c:c + w]))
        hg = 0.5 * g
        gate[c] = hg + hg * jnp.tanh(hg)

    def ffn_up(c, w):
        u = _dot(_bf(hn_s[...]), _bf(wu32[:, c:c + w]))
        act_s[:, c:c + w] = _pk(gate.pop(c) * u)

    def ffn_down(r, c, w):
        y = _dot(_bf(act_s[...]), _bf(wd32[:, c:c + w]))
        x_s[pl.ds(r, FB), c:c + w] = (x_s[pl.ds(r, FB), c:c + w].astype(F32) + y).astype(BF16)

    def out_copy(i):
        r = pl.ds(OUT_SPLIT[i], OUT_SPLIT[i + 1] - OUT_SPLIT[i])
        return pltpu.make_async_copy(x_s.at[r], out_hbm.at[r], sem_o.at[0])

    def iteration(u, mem, with_ffn):
        fill_a, fill_b, mid, end = {}, {}, [], []
        if with_ffn:
            @pl.when(u == OUT_SPLIT[1] // FB + 1)
            def _():
                out_copy(0).start()

            fr = pl.multiple_of(FB * u - FB, FB)
            ffn_ln(fr)
            ups = [functools.partial(f, c, 128) for c in range(0, FF, 128) for f in (ffn_gate, ffn_up)]
            downs = [functools.partial(ffn_down, fr, c, 128) for c in range(0, D, 128)]
            for t in UP_A:
                fill_a.setdefault(t, []).append(ups.pop(0))
            mid = [ups.pop(0) for _ in range(len(ups) - len(UP_B))]
            for t in UP_B:
                fill_b.setdefault(t, []).append(ups.pop(0))
            for t in DOWN_B:
                fill_b.setdefault(t, []).append(downs.pop(0))
            end = downs
        xn = [pool[NIT + i, :, 0:D] for i in range(4)]
        fill_a.setdefault(LN_AT, []).append(lambda: ln_next(jnp.minimum(FB * (u + 1), S - FB)))
        mem = step(xn[0], xn[1], mem, u, False, fill_a)
        for f in mid:
            f()
        mem = step(xn[2], xn[3], mem, u, True, fill_b)
        for f in end:
            f()
        return mem

    carry = iteration(0, mem_s[...].astype(F32), False)
    for c in f_copies:
        c.wait()
    jax.lax.fori_loop(1, NIT, functools.partial(iteration, with_ffn=True), carry)

    out_copy(1).start()
    ffn_ln(S - FB)
    for c in range(0, FF, FC):
        ffn_gate(c, FC)
        ffn_up(c, FC)
    ffn_down(S - FB, 0, D)
    out_copy(2).start()
    for i in range(3):
        out_copy(i).wait()


@jax.jit
def pallas_sequential_preLN__memory_aug_recurrent_mem_tr__swiglu_ffn__prompt_kernel(
    A_x: jax.Array,
    A_mem0: jax.Array,
    A_Wq: jax.Array,
    A_Wk: jax.Array,
    A_Wv: jax.Array,
    A_Wo: jax.Array,
    A_seg_len: jax.Array,
    B_x: jax.Array,
    B_w_gate: jax.Array,
    B_w_up: jax.Array,
    B_w_down: jax.Array,
):
    assert A_x.shape == (1, S, D) and A_Wq.shape == (D, H, DH) and A_mem0.shape == (1, M, D)
    x = A_x.reshape(S, D)
    mem0 = A_mem0.reshape(M, D)
    wq_t = A_Wq.transpose(1, 2, 0).reshape(H * DH, D)
    wk_t = A_Wk.transpose(1, 2, 0).reshape(H * DH, D)
    wv_t = A_Wv.transpose(1, 2, 0).reshape(H * DH, D)
    wo = A_Wo.reshape(H * DH, D)

    any_spec = pl.BlockSpec(memory_space=pl.ANY)
    out = pl.pallas_call(
        _kernel,
        in_specs=[any_spec] * 10,
        out_specs=any_spec,
        out_shape=jax.ShapeDtypeStruct((S, D), BF16),
        scratch_shapes=[
            pltpu.VMEM((S, D), BF16),
            pltpu.VMEM((NSEG, DQ, D), BF16),
            pltpu.VMEM((P0 // 2, D), U32),
            pltpu.VMEM((M, D), BF16),
            pltpu.VMEM((3, H * DH, D), BF16),
            pltpu.VMEM((D // 2, NP * QKVW), U32),
            pltpu.VMEM((H * DH // 2, D), U32),
            pltpu.VMEM((D // 2, FF), U32),
            pltpu.VMEM((D // 2, FF), U32),
            pltpu.VMEM((FF // 2, D), U32),
            pltpu.VMEM((NIT + 4, 8, NP * QKVW), U32),
            pltpu.VMEM(((SEG + M + DQ) // 2, H * DH), U32),
            pltpu.VMEM((2, 16, NP * QKVW), U32),
            pltpu.VMEM((FB // 2, D), U32),
            pltpu.VMEM((FB // 2, FF), U32),
            pltpu.SemaphoreType.DMA((6 + NPI,)),
            pltpu.SemaphoreType.DMA((1,)),
        ],
        compiler_params=pltpu.CompilerParams(vmem_limit_bytes=120 * 1024 * 1024),
    )(x, x.reshape(NSEG, SEG, D), mem0, wq_t, wk_t, wv_t, wo, B_w_gate, B_w_up, B_w_down)
    return out.reshape(1, S, D)
```

```python
import functools

import jax
import jax.numpy as jnp
import jax.experimental.pallas as pl
import jax.experimental.pallas.tpu as pltpu

F32 = jnp.float32
BF16 = jnp.bfloat16
U32 = jnp.uint32

S = 2048
D = 640
H = 32
DH = 192
M = 8
SEG = 32
NSEG = S // SEG
NIT = NSEG // 2
FF = 1536
NP = H // 2
PW = 2 * DH
QKVW = 3 * PW
DQ = 8
P0 = NSEG * DQ
PPI = 2
NPI = (NP - 2) // PPI
PM = 128
KPA, KPB = 48, 64
FB = 2 * SEG
FC = 512
OUT_SPLIT = (0, 28 * FB, S - FB, S)
EPS = 1e-5
LOG2E = 1.4426950408889634
LN_AT = 5
LAG_A = 3
LAG_B = 2
UP_A = tuple(range(1, 16)) + (("d", 2),)
UP_B = (1, 2, 3, 4, 5)
DOWN_B = (14, 15, ("d", 15))
EARLY_D = 10
D_FROM = 4
TAIL_A = (2, 2, 5, 9)
TAIL_B = (11, 12, 14)


def _ln(x):
    m = jnp.mean(x, axis=-1, keepdims=True)
    xc = x - m
    v = jnp.mean(xc * xc, axis=-1, keepdims=True)
    return xc * jax.lax.rsqrt(v + EPS)


def _dot(a, b):
    return jnp.dot(a, b, preferred_element_type=F32)


def _dot_nt(a, b):
    return jax.lax.dot_general(a, b, (((1,), (1,)), ((), ())),
                               preferred_element_type=F32)


def _bf(w32):
    return pltpu.bitcast(w32, BF16)


def _pk(x):
    return pltpu.bitcast(x.astype(BF16), U32)


def _halves(lo, hi):
    sub = jax.lax.broadcasted_iota(jnp.int32, lo.shape, 0)
    return jnp.where(sub < 4, lo, hi)


def _blockdiag(z32):
    n = z32.shape[0]
    lane = jax.lax.broadcasted_iota(jnp.int32, (n, 128), 1)
    mid = z32[:, 128:256]
    zero = jnp.zeros((n, 128), U32)
    top = jnp.concatenate([z32[:, :128], jnp.where(lane < 64, mid, zero), zero], axis=1)
    bot = jnp.concatenate([zero, jnp.where(lane >= 64, mid, zero), z32[:, 256:]], axis=1)
    return _bf(jnp.concatenate([top, bot], axis=0))


def _masks(odd):
    nq, kp = (SEG + M + DQ, KPB) if odd else (SEG - DQ + M, KPA)
    row = jax.lax.broadcasted_iota(jnp.int32, (nq, 128), 0)
    col = jax.lax.broadcasted_iota(jnp.int32, (nq, 128), 1)
    is_a = col < kp
    kc = jnp.where(is_a, col, col - kp)

    def pos(i):
        return jnp.where(i < 16, i + 16, jnp.where(i < 32, i - 16, i & 7))

    def between(i, lo, hi):
        return (i >= lo) & (i < hi)

    visible = between(kc, 16, 24) | (kc >= 48) | between(row, 16, 24) | (pos(kc) <= pos(row))
    if odd:
        prev_q = between(row, 32, 40)
        prev_k = between(kc, 32, 40) | between(kc, 48, 56)
        own_k = (kc < 32) | between(kc, 40, 48)
        is_key = (prev_q & prev_k) | (~prev_q & own_k)
    else:
        is_key = kc < 40
    return is_a, is_key, visible


def _kernel(x_hbm, x3_hbm, mem_hbm, wq_hbm, wk_hbm, wv_hbm, wo_hbm, wg_hbm, wu_hbm, wd_hbm,
            out_hbm,
            x_s, xl_s, xn_s, mem_s, stage, wo_st, wg_st, wu_st, wd_st, w32, wo32, pool,
            lo_s, cur_s, hn_s, act_s,
            sem, sem_o):
    w_hbms = (wq_hbm, wk_hbm, wv_hbm)

    def w_copy(j, m, n, k):
        rows = pl.ds(pl.multiple_of(j * PW, PW), n * PW)
        return pltpu.make_async_copy(w_hbms[m].at[rows], stage.at[m, rows], sem.at[k])

    x0_copy = pltpu.make_async_copy(x3_hbm.at[:, pl.ds(0, DQ), :], xl_s, sem.at[0])
    q0_copy = w_copy(0, 0, 1, 1)
    kv0_copies = [w_copy(0, m, 1, 2) for m in (1, 2)]
    p1_copies = [w_copy(1, m, 1, 3) for m in range(3)] + [
        pltpu.make_async_copy(x_hbm.at[pl.ds(0, FB)], x_s.at[pl.ds(0, FB)], sem.at[3])]
    x1_copy = pltpu.make_async_copy(x_hbm.at[pl.ds(FB, S - FB)], x_s.at[pl.ds(FB, S - FB)], sem.at[4])
    mem_copy = pltpu.make_async_copy(mem_hbm, mem_s, sem.at[4])
    of_copies = [pltpu.make_async_copy(src, dst, sem.at[4])
                 for src, dst in ((wo_hbm, wo_st), (wg_hbm, wg_st), (wu_hbm, wu_st), (wd_hbm, wd_st))]

    def group_copies(i):
        return [w_copy(2 + PPI * i, m, PPI, 5 + i) for m in range(3)]

    for c in [x0_copy, q0_copy] + kv0_copies + p1_copies:
        c.start()
    for i in range(NPI):
        for c in group_copies(i):
            c.start()
        if i == 0:
            x1_copy.start()
            mem_copy.start()

    x0_copy.wait()
    for g in range(0, NSEG, 16):
        xl = xl_s[g:g + 16].astype(F32).reshape(128, D)
        xn_s[4 * g:4 * g + 64, :] = _pk(_ln(xl))

    def ln_next(t):
        xn = _pk(_ln(x_s[pl.ds(pl.multiple_of(t, FB), FB), :].astype(F32)))
        pool[NIT:NIT + 4, :, 0:D] = xn.reshape(4, 8, D)

    def chunk(j, m):
        wt = stage[m, pl.ds(pl.multiple_of(j * PW, PW), PW), :]
        col = pl.ds(pl.multiple_of(j * QKVW + m * PW, 128), PW)
        for r in range(0, P0, PM):
            y = _dot_nt(_bf(xn_s[r // 2:(r + PM) // 2, :]), wt)
            pool[r // 16:(r + PM) // 16, :, col] = _pk(y).reshape(PM // 16, 8, PW)
        w32[:, col] = pltpu.bitcast(wt.T, U32)

    q0_copy.wait()
    chunk(0, 0)
    for c in kv0_copies:
        c.wait()
    chunk(0, 1)
    chunk(0, 2)
    for c in p1_copies:
        c.wait()
    ln_next(0)
    for m in range(3):
        chunk(1, m)
    for c in of_copies:
        c.start()

    def prologue(i, carry):
        for c in group_copies(i):
            c.wait()
        for jj in range(PPI):
            for m in range(3):
                chunk(2 + PPI * i + jj, m)
        return carry

    jax.lax.fori_loop(0, NPI, prologue, 0)
    for c in [x1_copy, mem_copy] + of_copies:
        c.wait()

    scale = DH ** -0.5
    neg_inf = float("-inf")

    def step(xn_lo, xn_hi, mem, u, odd, fillers, first=False):
        mem_pk = _pk(jnp.concatenate([mem, jnp.zeros((8, D), F32)], axis=0))
        lhs = _bf(jnp.concatenate([xn_hi, _halves(mem_pk, xn_lo)], axis=0))
        nq = SEG + M + DQ if odd else SEG - DQ + M
        is_a, is_key, visible = _masks(odd)
        p = {}

        def stage_a(j):
            cs = slice(j * QKVW, (j + 1) * QKVW)
            cur_s[int(odd), :, cs] = _pk(_dot(lhs, _bf(w32[:, cs])))

        def tok(j, m):
            if m == 0 and not odd:
                return None
            return pool[u, :, j * QKVW + m * PW:j * QKVW + (m + 1) * PW]

        def rows(lead, j, m):
            cs = slice(j * QKVW + m * PW, j * QKVW + (m + 1) * PW)
            zero = jnp.zeros((8, PW), U32)
            parts = [cur_s[int(odd), :, cs]]
            if odd:
                parts.append(lead)
                if m:
                    parts.append(_halves(cur_s[0, 8:16, cs], zero))
            elif m:
                parts.append(_halves(lead, zero))
            return jnp.concatenate(parts, axis=0)

        def stage_b(j, qt, kt):
            sc = _dot_nt(_bf(rows(qt, j, 0)), _blockdiag(rows(kt, j, 1)))
            sc = sc * (scale * LOG2E)
            nk = sc.shape[1]
            if nk < 128:
                sc = jnp.concatenate([sc, jnp.full((nq, 128 - nk), neg_inf, F32)], axis=1)
            sc = jnp.where(visible, sc, -1e9 * LOG2E)
            sc = jnp.where(is_key, sc, neg_inf)
            ma = jnp.max(jnp.where(is_a, sc, neg_inf), axis=1, keepdims=True)
            mb = jnp.max(jnp.where(is_a, neg_inf, sc), axis=1, keepdims=True)
            e = jnp.exp2(sc - jnp.where(is_a, ma, mb))
            sa = jnp.sum(jnp.where(is_a, e, 0.0), axis=1, keepdims=True)
            sb = jnp.sum(jnp.where(is_a, 0.0, e), axis=1, keepdims=True)
            den = jnp.where(is_a, sa, sb)
            r = pl.reciprocal(den, approx=True)
            p[j] = (e * (r * (2.0 - den * r)))[:, 0:nk].astype(BF16)

        def stage_c(j, vt):
            o = _dot(p[j], _blockdiag(rows(vt, j, 2)))
            lo_s[0:nq // 2, j * PW:(j + 1) * PW] = _pk(o)

        def stage_d(j, acc):
            wrows = slice(j * (PW // 2), (j + 1) * (PW // 2))
            if first:
                w = wo_st[j * PW:(j + 1) * PW, :]
                wo32[wrows, :] = pltpu.bitcast(w, U32)
            else:
                w = _bf(wo32[wrows, :])
            d = _dot(_bf(lo_s[0:nq // 2, j * PW:(j + 1) * PW]), w)
            return d if acc is None else acc + d

        def fill(key):
            for f in fillers.get(key, ()):
                f()

        acc, nd = None, 0
        lag = LAG_B if odd else LAG_A
        for t in range(NP):
            if t >= 1:
                qt, kt = tok(t - 1, 0), tok(t - 1, 1)
            if t >= lag:
                vt = tok(t - lag, 2)
            stage_a(t)
            fill(t)
            if odd and t >= D_FROM and nd < EARLY_D:
                acc = stage_d(nd, acc)
                nd += 1
            if t >= 1:
                stage_b(t - 1, qt, kt)
            if t >= lag:
                stage_c(t - lag, vt)
        tail = TAIL_B if odd else TAIL_A
        for j in range(nd, NP):
            if j == tail[0]:
                stage_b(NP - 1, tok(NP - 1, 0), tok(NP - 1, 1))
            for i in range(lag):
                if j == tail[1 + i]:
                    stage_c(NP - lag + i, tok(NP - lag + i, 2))
            fill(("d", j))
            acc = stage_d(j, acc)

        def residual(t, a):
            hr = pl.ds(pl.multiple_of(t, 8), a.shape[0])
            x_s[hr, :] = (x_s[hr, :].astype(F32) + a).astype(BF16)

        t0 = FB * u + SEG if odd else FB * u
        residual(t0 + 16, acc[0:16])
        residual(t0 + 8, acc[24:32])
        if odd:
            residual(t0 - SEG, acc[32:40])
            residual(t0, acc[40:48])
        return acc[16:24]

    def ffn_ln(r):
        hn_s[...] = _pk(_ln(x_s[pl.ds(r, FB), :].astype(F32)))

    gate = {}

    def ffn_gate(c, w):
        g = _dot(_bf(hn_s[...]), wg_st[:, c:c + w])
        hg = 0.5 * g
        gate[c] = hg + hg * jnp.tanh(hg)

    def ffn_up(c, w):
        u = _dot(_bf(hn_s[...]), wu_st[:, c:c + w])
        act_s[:, c:c + w] = _pk(gate.pop(c) * u)

    def ffn_down(r, c, w):
        y = _dot(_bf(act_s[...]), wd_st[:, c:c + w])
        x_s[pl.ds(r, FB), c:c + w] = (x_s[pl.ds(r, FB), c:c + w].astype(F32) + y).astype(BF16)

    def out_copy(i):
        r = pl.ds(OUT_SPLIT[i], OUT_SPLIT[i + 1] - OUT_SPLIT[i])
        return pltpu.make_async_copy(x_s.at[r], out_hbm.at[r], sem_o.at[0])

    def iteration(u, mem, with_ffn):
        fill_a, fill_b, mid, end = {}, {}, [], []
        if with_ffn:
            @pl.when(u == OUT_SPLIT[1] // FB + 1)
            def _():
                out_copy(0).start()

            fr = pl.multiple_of(FB * u - FB, FB)
            ffn_ln(fr)
            ups = [functools.partial(f, c, 128) for c in range(0, FF, 128) for f in (ffn_gate, ffn_up)]
            downs = [functools.partial(ffn_down, fr, c, 128) for c in range(0, D, 128)]
            for t in UP_A:
                fill_a.setdefault(t, []).append(ups.pop(0))
            mid = [ups.pop(0) for _ in range(len(ups) - len(UP_B))]
            for t in UP_B:
                fill_b.setdefault(t, []).append(ups.pop(0))
            for t in DOWN_B:
                fill_b.setdefault(t, []).append(downs.pop(0))
            end = downs
        xn = [pool[NIT + i, :, 0:D] for i in range(4)]
        fill_a.setdefault(LN_AT, []).append(lambda: ln_next(jnp.minimum(FB * (u + 1), S - FB)))
        mem = step(xn[0], xn[1], mem, u, False, fill_a, first=not with_ffn)
        for f in mid:
            f()
        mem = step(xn[2], xn[3], mem, u, True, fill_b)
        for f in end:
            f()
        return mem

    carry = iteration(0, mem_s[...].astype(F32), False)
    jax.lax.fori_loop(1, NIT, functools.partial(iteration, with_ffn=True), carry)

    out_copy(1).start()
    ffn_ln(S - FB)
    for c in range(0, FF, FC):
        ffn_gate(c, FC)
        ffn_up(c, FC)
    ffn_down(S - FB, 0, D)
    out_copy(2).start()
    for i in range(3):
        out_copy(i).wait()


@jax.jit
def pallas_sequential_preLN__memory_aug_recurrent_mem_tr__swiglu_ffn__prompt_kernel(
    A_x: jax.Array,
    A_mem0: jax.Array,
    A_Wq: jax.Array,
    A_Wk: jax.Array,
    A_Wv: jax.Array,
    A_Wo: jax.Array,
    A_seg_len: jax.Array,
    B_x: jax.Array,
    B_w_gate: jax.Array,
    B_w_up: jax.Array,
    B_w_down: jax.Array,
):
    assert A_x.shape == (1, S, D) and A_Wq.shape == (D, H, DH) and A_mem0.shape == (1, M, D)
    x = A_x.reshape(S, D)
    mem0 = A_mem0.reshape(M, D)
    wq_t = A_Wq.transpose(1, 2, 0).reshape(H * DH, D)
    wk_t = A_Wk.transpose(1, 2, 0).reshape(H * DH, D)
    wv_t = A_Wv.transpose(1, 2, 0).reshape(H * DH, D)
    wo = A_Wo.reshape(H * DH, D)

    any_spec = pl.BlockSpec(memory_space=pl.ANY)
    out = pl.pallas_call(
        _kernel,
        in_specs=[any_spec] * 10,
        out_specs=any_spec,
        out_shape=jax.ShapeDtypeStruct((S, D), BF16),
        scratch_shapes=[
            pltpu.VMEM((S, D), BF16),
            pltpu.VMEM((NSEG, DQ, D), BF16),
            pltpu.VMEM((P0 // 2, D), U32),
            pltpu.VMEM((M, D), BF16),
            pltpu.VMEM((3, H * DH, D), BF16),
            pltpu.VMEM((H * DH, D), BF16),
            pltpu.VMEM((D, FF), BF16),
            pltpu.VMEM((D, FF), BF16),
            pltpu.VMEM((FF, D), BF16),
            pltpu.VMEM((D // 2, NP * QKVW), U32),
            pltpu.VMEM((H * DH // 2, D), U32),
            pltpu.VMEM((NIT + 4, 8, NP * QKVW), U32),
            pltpu.VMEM(((SEG + M + DQ) // 2, H * DH), U32),
            pltpu.VMEM((2, 16, NP * QKVW), U32),
            pltpu.VMEM((FB // 2, D), U32),
            pltpu.VMEM((FB // 2, FF), U32),
            pltpu.SemaphoreType.DMA((5 + NPI,)),
            pltpu.SemaphoreType.DMA((1,)),
        ],
        compiler_params=pltpu.CompilerParams(vmem_limit_bytes=120 * 1024 * 1024),
    )(x, x.reshape(NSEG, SEG, D), mem0, wq_t, wk_t, wv_t, wo, B_w_gate, B_w_up, B_w_down)
    return out.reshape(1, S, D)
```
